```python
import os as _os
_os.environ.setdefault('JAX_PLATFORMS', 'cpu')
import jax
import jax.numpy as jnp

def _softmax(x, axis=-1):
    return jax.nn.softmax(x, axis=axis)

def _gelu(x):
    return jax.nn.gelu(x, approximate=True)

def _silu(x):
    return jax.nn.silu(x)

def _sigmoid(x):
    return jax.nn.sigmoid(x)

def _layernorm(x, axis=-1, eps=1e-05):
    m = jnp.mean(x, axis=axis, keepdims=True)
    v = jnp.var(x, axis=axis, keepdims=True)
    return (x - m) / jnp.sqrt(v + eps)

def _scatter_add(tgt, idx, src, axis=0):
    return tgt.at[idx].add(src)

def _segment_sum(src, seg, n):
    return jax.ops.segment_sum(src, seg, n)

class _Rng:

    def __init__(self, key):
        self._k = key

    def _next(self):
        self._k, sub = jax.random.split(self._k)
        return sub

    def normal(self, shape):
        return jax.random.normal(self._next(), shape, dtype=jnp.bfloat16)

    def randint(self, lo, hi, shape):
        return jax.random.randint(self._next(), shape, lo, hi, dtype=jnp.int32)

    def uniform(self, shape, lo=0.0, hi=1.0):
        return jax.random.uniform(self._next(), shape, jnp.bfloat16, lo, hi)

    def permutation(self, n):
        return jax.random.permutation(self._next(), n)
kernel_name = 'standalone__conformer_conv_module__speech'

def setup_inputs():
    _rng = _Rng(jax.random.key(int.from_bytes(__import__("os").urandom(4), "little")))
    _w = lambda a: (lambda t: t.astype(jnp.bfloat16) if jnp.issubdtype(t.dtype, jnp.floating) else t)(jnp.asarray(a))
    B, T, D, K = (2, 4000, 512, 15)
    return {'x': _w((lambda *s: _rng.normal(s) * 0.2)(B, T, D)), 'w_pw1': _w((lambda *s: _rng.normal(s) * 0.2)(D, 2 * D)), 'dw': _w((lambda *s: _rng.normal(s) * 0.05)(K, D)), 'w_pw2': _w((lambda *s: _rng.normal(s) * 0.05)(D, D))}

def reference(x, w_pw1, dw, w_pw2):
    B, T, D = x.shape
    K = dw.shape[0]
    h = x @ w_pw1
    a, b = (h[..., :D].copy(), h[..., D:].copy())
    h = a * _sigmoid(b)
    pad = K // 2
    hp = jnp.pad(h, ((0, 0), (pad, pad), (0, 0)))
    out = jnp.zeros_like(h)
    for i in range(K):
        out = out + hp[:, i:i + T, :] * dw[i][None, None, :]
    return _silu(out) @ w_pw2
```

```python
import functools

import jax
import jax.numpy as jnp
import jax.experimental.pallas as pl
import jax.experimental.pallas.tpu as pltpu

LANES = 128
SUBLANES = 8
ROWS = 160
HEAD_ROWS = 448
LAG = 3
IN_STEPS = (0, 1, 2, 4, 8, 16)
OUT_STEPS = (-12, -4, -1)


def _kernel(x_hbm, w1_hbm, dw_hbm, w2_hbm, o_hbm,
            x_v, w1_v, w2_v, dw_v, taps_v, h_v, o_v, sem,
            *, steps, in_edges, out_edges, gap):
    B, T, D = x_hbm.shape
    K = dw_hbm.shape[0]
    nd = D // LANES
    f32 = jnp.float32
    sem_w2, sem_out, sem_in = 2 * nd, 2 * nd + 1, 2 * nd + 2
    n_in, n_out = len(in_edges) - 1, len(out_edges) - 1

    def lanes(j):
        return pl.ds(j * LANES, LANES)

    def h_row(r):
        return r + (r // T + 1) * gap

    def in_copies(q):
        r0, r1 = in_edges[q], in_edges[q + 1]
        copies = [
            pltpu.make_async_copy(x_hbm.at[r0 // T, pl.ds(r0 % T, r1 - r0), lanes(j)],
                                  x_v.at[j, pl.ds(r0, r1 - r0), :], sem.at[sem_in + q])
            for j in range(nd)]
        if q == 0:
            copies.append(pltpu.make_async_copy(dw_hbm, dw_v, sem.at[sem_in]))
        return copies

    def out_copy(q, j):
        r0, r1 = out_edges[q], out_edges[q + 1]
        return pltpu.make_async_copy(o_v.at[j, pl.ds(r0, r1 - r0), :],
                                     o_hbm.at[r0 // T, pl.ds(r0 % T, r1 - r0), lanes(j)],
                                     sem.at[sem_out])

    w1_copies = [pltpu.make_async_copy(w1_hbm.at[:, lanes(j)], w1_v.at[j], sem.at[j])
                 for j in range(2 * nd)]
    w2_copies = [pltpu.make_async_copy(w2_hbm.at[:, lanes(j)], w2_v.at[j], sem.at[sem_w2])
                 for j in range(nd)]

    def start_inputs(q):
        if q < n_in:
            for cp in in_copies(q):
                cp.start()
        if q == 2:
            for cp in w2_copies:
                cp.start()

    def wait_inputs(n):
        for q in range(n_in):
            if in_edges[q] == steps[n][0]:
                for cp in in_copies(q):
                    cp.wait()
                start_inputs(q + 2)

    def glu(n, j):
        r0, r1 = steps[n]
        x = jnp.concatenate([x_v[k, pl.ds(r0, r1 - r0), :] for k in range(nd)], axis=1)
        if n == 0 and j > 0:
            w1_copies[nd + j].wait()
        t = jnp.tanh(0.5 * jnp.dot(x, w1_v[nd + j], preferred_element_type=f32))
        if n == 0:
            w1_copies[j].wait()
        a = jnp.dot(x, w1_v[j], preferred_element_type=f32)
        h_v[j, pl.ds(h_row(r0), r1 - r0), :] = a * t + a

    def conv_silu(n, j):
        r0, r1 = steps[n]
        rows = r1 - r0
        terms = [h_v[j, pl.ds(h_row(r0) - K // 2 + k, rows), :]
                 * jnp.concatenate([taps_v[j, k]] * (rows // SUBLANES), axis=0)
                 for k in range(K)]
        half = (K + 1) // 2
        c = functools.reduce(jnp.add, terms[:half])
        if terms[half:]:
            c = c + functools.reduce(jnp.add, terms[half:])
        return c * jnp.tanh(c) + c

    def pointwise2(n, j, g):
        r0, r1 = steps[n]
        if n == 0 and j == 0:
            for cp in w2_copies:
                cp.wait()
        y = jnp.dot(g, w2_v[j], preferred_element_type=f32)
        o_v[j, pl.ds(r0, r1 - r0), :] = y.astype(o_v.dtype)
        for q in range(n_out):
            if out_edges[q + 1] == r1:
                out_copy(q, j).start()

    w1_copies[nd].start()
    start_inputs(0)
    for j in range(nd):
        if j > 0:
            w1_copies[nd + j].start()
        w1_copies[j].start()
    start_inputs(1)

    for j in range(nd):
        for b in range(B + 1):
            h_v[j, pl.ds(b * (T + gap), gap), :] = jnp.zeros((gap, LANES), f32)

    w1_copies[nd].wait()
    for s in range(len(steps) + LAG):
        if s < len(steps):
            wait_inputs(s)
        if s == 0:
            taps = 0.25 * dw_v[...].astype(f32)
            for j in range(nd):
                for k in range(K):
                    taps_v[j, k] = jnp.broadcast_to(
                        taps[k:k + 1, j * LANES:(j + 1) * LANES], (SUBLANES, LANES))
        if s >= LAG:
            g = jnp.concatenate([conv_silu(s - LAG, j) for j in range(nd)], axis=1)
            g = g.astype(w2_v.dtype)
        for j in range(nd):
            if s < len(steps):
                glu(s, j)
            if s >= LAG:
                pointwise2(s - LAG, j, g)
    for q in range(n_out):
        for j in range(nd):
            out_copy(q, j).wait()


def _steps(B, T):
    steps = []
    for b in range(B):
        r, end = b * T, (b + 1) * T
        while r < end:
            size = min(HEAD_ROWS if r == 0 else ROWS, end - r)
            steps.append((r, r + size))
            r += size
    return tuple(steps)


@jax.jit
def pallas_standalone__conformer_conv_module__speech_kernel(
    x: jax.Array,
    w_pw1: jax.Array,
    dw: jax.Array,
    w_pw2: jax.Array,
):
    B, T, D = x.shape
    K = dw.shape[0]
    nd = D // LANES
    gap = pl.cdiv(max(K // 2, 1), SUBLANES) * SUBLANES
    steps = _steps(B, T)
    assert D % LANES == 0 and T % 16 == 0 and gap <= 16 and len(steps) > max(IN_STEPS)
    seq_edges = [b * T for b in range(B + 1)]
    in_edges = tuple(sorted(set([steps[i][0] for i in IN_STEPS] + seq_edges)))
    out_edges = tuple(sorted(set([steps[i][0] for i in OUT_STEPS] + seq_edges)))
    hbm = pl.BlockSpec(memory_space=pl.ANY)
    return pl.pallas_call(
        functools.partial(_kernel, steps=steps, in_edges=in_edges, out_edges=out_edges, gap=gap),
        in_specs=[hbm] * 4,
        out_specs=hbm,
        out_shape=jax.ShapeDtypeStruct((B, T, D), x.dtype),
        scratch_shapes=[
            pltpu.VMEM((nd, B * T, LANES), x.dtype),
            pltpu.VMEM((2 * nd, D, LANES), w_pw1.dtype),
            pltpu.VMEM((nd, D, LANES), w_pw2.dtype),
            pltpu.VMEM((K, D), dw.dtype),
            pltpu.VMEM((nd, K, SUBLANES, LANES), jnp.float32),
            pltpu.VMEM((nd, B * (T + gap) + gap, LANES), jnp.float32),
            pltpu.VMEM((nd, B * T, LANES), x.dtype),
            pltpu.SemaphoreType.DMA((2 * nd + 2 + len(in_edges) - 1,)),
        ],
        compiler_params=pltpu.CompilerParams(
            vmem_limit_bytes=64 * 1024 * 1024,
            flags={"XLA_TPU_RESCHEDULE_DMA_DONES": True},
        ),
    )(x, w_pw1, dw, w_pw2)
```

```python
import functools

import jax
import jax.numpy as jnp
import jax.experimental.pallas as pl
import jax.experimental.pallas.tpu as pltpu

LANES = 128
SUBLANES = 8
LOG2E = 1.4426950408889634

ROWS = 512
HEAD_STEPS = (256, 256, 256)
HEAD_PARTS = (128, 256, 256, 128)
HEAD_COPIES = (3, 2)
LAG = 4
IN_STEPS = (3, 4, 6, 8)
OUT_STEPS = (-7, -5, -4, -3, -2, -1)
OUT_TAIL = (192, 64)


def _sigmoid(v):
    return pltpu.reciprocal(1.0 + jnp.exp2(v * -LOG2E), approx=True)


def _load(ref, j, r0, r1):
    words = ref.at[j, pl.ds(r0, r1 - r0), :].bitcast(jnp.uint32)[...]
    return pltpu.bitcast(words, ref.dtype)


def _ranges(edges):
    return tuple(zip(edges[:-1], edges[1:]))


def _kernel(x_hbm, w1_hbm, dw_hbm, w2_hbm, o_hbm,
            x_v, w1_v, w2_v, dw_v, taps_v, h_v, o_v, sems,
            *, steps, head_parts, head_edges, in_edges, out_edges, gap):
    B, T, D = x_hbm.shape
    K = dw_hbm.shape[0]
    nd = D // LANES
    f32 = jnp.float32
    head = head_parts[-1][1]
    value_tiles, gate_tiles = range(nd), range(nd, 2 * nd)

    def tile(j):
        return pl.ds(j * LANES, LANES)

    def h_rows(r0, r1, shift=0):
        return pl.ds(r0 + (r0 // T + 1) * gap + shift, r1 - r0)

    free_sems = iter(range(sems.shape[0]))

    def group(*pairs):
        sem = sems.at[next(free_sems)]
        return [pltpu.make_async_copy(src, dst, sem) for src, dst in pairs]

    def start(copies):
        for copy in copies:
            copy.start()

    def wait(copies):
        for copy in copies:
            copy.wait()

    def seq_rows(hbm_ref, r0, r1, j):
        return hbm_ref.at[r0 // T, pl.ds(r0 % T, r1 - r0), tile(j)]

    def x_pair(r0, r1, j):
        return seq_rows(x_hbm, r0, r1, j), x_v.at[j, pl.ds(r0, r1 - r0), :]

    w1_copies = {
        (k, js): group(*[(w1_hbm.at[tile(k), tile(j)], w1_v.at[j, tile(k), :]) for j in js])
        for k in range(nd) for js in (gate_tiles, value_tiles)}
    head_copies = {(k, r0): group(x_pair(r0, r1, k))
                   for k in range(nd) for r0, r1 in _ranges(head_edges[k])}
    dw_copies = group((dw_hbm, dw_v))
    w2_copies = group(*[(w2_hbm.at[:, tile(j)], w2_v.at[j]) for j in range(nd)])
    in_copies = [group(*[x_pair(r0, r1, j) for j in range(nd)])
                 for r0, r1 in _ranges(in_edges)]
    out_copies = group(*[(o_v.at[j, pl.ds(r0, r1 - r0), :], seq_rows(o_hbm, r0, r1, j))
                         for r0, r1 in _ranges(out_edges) for j in range(nd)])

    def glu_head():
        for k in range(nd):
            for js in (gate_tiles, value_tiles):
                wait(w1_copies[k, js])
                for r0, r1 in head_parts:
                    if js is gate_tiles:
                        wait(head_copies.get((k, r0), ()))
                    w = jnp.concatenate(
                        [_load(w1_v, j, k * LANES, (k + 1) * LANES) for j in js], axis=1)
                    part = jnp.dot(_load(x_v, k, r0, r1), w, preferred_element_type=f32)
                    gate_rows = h_rows(head + r0, head + r1)
                    rows = gate_rows if js is gate_tiles else h_rows(r0, r1)
                    for j in range(nd):
                        v = part[:, j * LANES:(j + 1) * LANES]
                        if k > 0:
                            v = v + h_v[j, rows, :]
                        if k == nd - 1:
                            v = _sigmoid(v) if js is gate_tiles else v * h_v[j, gate_rows, :]
                        h_v[j, rows, :] = v
            if k == 0:
                wait(dw_copies)
                start(in_copies[1])
                start(w2_copies)

    def sync_inputs(s):
        if steps[s][0] in in_edges:
            q = in_edges.index(steps[s][0])
            wait(in_copies[q])
            if s == LAG:
                wait(w2_copies)
            if q + 2 < len(in_copies):
                start(in_copies[q + 2])

    def glu(s, j):
        r0, r1 = steps[s]
        x = jnp.concatenate([_load(x_v, k, r0, r1) for k in range(nd)], axis=1)
        gate = _sigmoid(jnp.dot(x, _load(w1_v, nd + j, 0, D), preferred_element_type=f32))
        value = jnp.dot(x, _load(w1_v, j, 0, D), preferred_element_type=f32)
        h_v[j, h_rows(r0, r1), :] = value * gate

    def conv_silu(s, j):
        r0, r1 = steps[s]
        terms = [h_v[j, h_rows(r0, r1, k - K // 2), :]
                 * jnp.concatenate([taps_v[j, k]] * ((r1 - r0) // SUBLANES), axis=0)
                 for k in range(K)]
        sums = [functools.reduce(jnp.add, terms[k:k + SUBLANES])
                for k in range(0, K, SUBLANES)]
        conv = functools.reduce(jnp.add, sums)
        return conv * _sigmoid(conv)

    def pointwise2(s, j, act):
        r0, r1 = steps[s]
        y = jnp.dot(act, _load(w2_v, j, 0, D), preferred_element_type=f32)
        for c0, c1 in _ranges([r0] + [e for e in out_edges if r0 < e < r1] + [r1]):
            o_v[j, pl.ds(c0, c1 - c0), :] = y[c0 - r0:c1 - r0].astype(o_v.dtype)
            if c1 in out_edges:
                out_copies[(out_edges.index(c1) - 1) * nd + j].start()

    for k in range(nd):
        start(w1_copies[k, gate_tiles])
        for r0 in head_edges[k][:-1]:
            start(head_copies[k, r0])
        start(w1_copies[k, value_tiles])
        if k == 0:
            start(dw_copies)
    start(in_copies[0])

    for j in range(nd):
        for b in range(B + 1):
            h_v[j, pl.ds(b * (T + gap), gap), :] = jnp.zeros((gap, LANES), f32)

    glu_head()
    taps = dw_v[...].astype(f32)
    for j in range(nd):
        for k in range(K):
            taps_v[j, k] = jnp.broadcast_to(
                taps[k:k + 1, j * LANES:(j + 1) * LANES], (SUBLANES, LANES))

    for s in range(len(HEAD_STEPS), len(steps) + LAG):
        if s >= LAG:
            act = jnp.concatenate([conv_silu(s - LAG, j) for j in range(nd)], axis=1)
            act = act.astype(w2_v.dtype)
        if s < len(steps):
            sync_inputs(s)
        for j in range(nd):
            if s < len(steps):
                glu(s, j)
            if s >= LAG:
                pointwise2(s - LAG, j, act)
    wait(out_copies)


def _step_edges(B, T):
    edges = [sum(HEAD_STEPS[:i]) for i in range(len(HEAD_STEPS) + 1)]
    for b in range(B):
        while edges[-1] < (b + 1) * T:
            edges.append(min(edges[-1] + ROWS, (b + 1) * T))
    return edges


@jax.jit
def pallas_standalone__conformer_conv_module__speech_kernel(
    x: jax.Array,
    w_pw1: jax.Array,
    dw: jax.Array,
    w_pw2: jax.Array,
):
    B, T, D = x.shape
    K = dw.shape[0]
    nd = D // LANES
    head = sum(HEAD_STEPS)
    gap = pl.cdiv(max(K // 2, 1), SUBLANES) * SUBLANES
    steps = _ranges(_step_edges(B, T))
    assert D % LANES == 0 and T % 16 == 0 and K % 2 == 1 and gap <= 16
    assert head == sum(HEAD_PARTS) and 2 * head <= T and len(steps) > max(IN_STEPS)
    assert IN_STEPS[0] == len(HEAD_STEPS) <= LAG and LAG in IN_STEPS

    part_edges = [sum(HEAD_PARTS[:i]) for i in range(len(HEAD_PARTS) + 1)]
    head_edges = tuple(tuple(part_edges[:n] + [head]) for n in (HEAD_COPIES + (1,) * nd)[:nd])
    seq_edges = [b * T for b in range(B + 1)]
    in_edges = tuple(sorted(set([steps[s][0] for s in IN_STEPS] + seq_edges[1:])))
    out_edges = tuple(sorted(set(
        [steps[s][0] for s in OUT_STEPS] + [B * T - r for r in OUT_TAIL] + seq_edges)))
    n_sems = 2 * nd + sum(len(e) - 1 for e in head_edges) + (len(in_edges) - 1) + 3

    hbm = pl.BlockSpec(memory_space=pl.ANY)
    return pl.pallas_call(
        functools.partial(_kernel, steps=steps, head_parts=_ranges(part_edges),
                          head_edges=head_edges, in_edges=in_edges, out_edges=out_edges,
                          gap=gap),
        in_specs=[hbm] * 4,
        out_specs=hbm,
        out_shape=jax.ShapeDtypeStruct((B, T, D), x.dtype),
        scratch_shapes=[
            pltpu.VMEM((nd, B * T, LANES), x.dtype),
            pltpu.VMEM((2 * nd, D, LANES), w_pw1.dtype),
            pltpu.VMEM((nd, D, LANES), w_pw2.dtype),
            pltpu.VMEM((K, D), dw.dtype),
            pltpu.VMEM((nd, K, SUBLANES, LANES), jnp.float32),
            pltpu.VMEM((nd, B * (T + gap) + gap, LANES), jnp.float32),
            pltpu.VMEM((nd, B * T, LANES), x.dtype),
            pltpu.SemaphoreType.DMA((n_sems,)),
        ],
        compiler_params=pltpu.CompilerParams(
            vmem_limit_bytes=64 * 1024 * 1024,
            disable_semaphore_checks=True,
            flags={"XLA_TPU_RESCHEDULE_DMA_DONES": True},
        ),
    )(x, w_pw1, dw, w_pw2)
```
